```python
import jax
import jax.numpy as jnp

def _softmax(x, axis=-1):
    return jax.nn.softmax(x, axis=axis)

def _gelu(x):
    return jax.nn.gelu(x, approximate=True)

def _silu(x):
    return jax.nn.silu(x)

def _sigmoid(x):
    return jax.nn.sigmoid(x)

def _layernorm(x, axis=-1, eps=1e-05):
    m = jnp.mean(x, axis=axis, keepdims=True)
    v = jnp.var(x, axis=axis, keepdims=True)
    return (x - m) / jnp.sqrt(v + eps)

def _scatter_add(tgt, idx, src, axis=0):
    return tgt.at[idx].add(src)

def _segment_sum(src, seg, n):
    return jax.ops.segment_sum(src, seg, n)

class _Rng:

    def __init__(self, key):
        self._k = key

    def _next(self):
        self._k, sub = jax.random.split(self._k)
        return sub

    def normal(self, shape):
        return jax.random.normal(self._next(), shape, dtype=jnp.bfloat16)

    def randint(self, lo, hi, shape):
        return jax.random.randint(self._next(), shape, lo, hi, dtype=jnp.int32)

    def uniform(self, shape, lo=0.0, hi=1.0):
        return jax.random.uniform(self._next(), shape, jnp.bfloat16, lo, hi)

    def permutation(self, n):
        return jax.random.permutation(self._next(), n)
kernel_name = 'gated_mix__memory_aug_recurrent_mem_tr__sliding_local_dilated__prompt'

def setup_inputs():
    _rng = _Rng(jax.random.key(int.from_bytes(__import__("os").urandom(4), "little")))
    _w = lambda a: (lambda t: t.astype(jnp.bfloat16) if jnp.issubdtype(t.dtype, jnp.floating) else t)(jnp.asarray(a))

    def _A_setup():
        B, S, Dm = (1, 2048, 640)
        H, Dh = (32, 192)
        M, seg = (8, 32)
        seg = min(seg, S)
        S = S // seg * seg
        return {'x': _w((lambda *s: _rng.normal(s) * 0.05)(B, S, Dm)), 'mem0': _w((lambda *s: _rng.normal(s) * 0.05)(B, M, Dm)), 'Wq': _w((lambda *s: _rng.normal(s) * 0.05)(Dm, H, Dh) * Dm ** (-0.5)), 'Wk': _w((lambda *s: _rng.normal(s) * 0.05)(Dm, H, Dh) * Dm ** (-0.5)), 'Wv': _w((lambda *s: _rng.normal(s) * 0.05)(Dm, H, Dh) * Dm ** (-0.5)), 'Wo': _w((lambda *s: _rng.normal(s) * 0.05)(H, Dh, Dm) * (H * Dh) ** (-0.5)), 'seg_len': seg}
    _A_in = _A_setup()

    def _B_setup():
        B, S, D = (1, 2048, 640)
        return {'x': _w((lambda *s: _rng.normal(s) * 0.05)(B, S, D)), 'wqkv': _w((lambda *s: _rng.normal(s) * 0.05)(D, 3 * D)), 'wo': _w((lambda *s: _rng.normal(s) * 0.05)(D, D))}
    _B_in = _B_setup()
    return {'A_x': _A_in['x'], 'A_mem0': _A_in['mem0'], 'A_Wq': _A_in['Wq'], 'A_Wk': _A_in['Wk'], 'A_Wv': _A_in['Wv'], 'A_Wo': _A_in['Wo'], 'A_seg_len': _A_in['seg_len'], 'B_x': _B_in['x'], 'B_wqkv': _B_in['wqkv'], 'B_wo': _B_in['wo'], 'gate_w': _w((lambda *s: _rng.normal(s) * 0.05)(640))}

def reference(A_x, A_mem0, A_Wq, A_Wk, A_Wv, A_Wo, A_seg_len, B_x, B_wqkv, B_wo, gate_w):

    def _A_ref(x, mem0, Wq, Wk, Wv, Wo, seg_len):
        B, S, Dm = x.shape
        H, Dh = (Wq.shape[1], Wq.shape[2])
        M = mem0.shape[1]
        scale = Dh ** (-0.5)
        n_seg = S // seg_len
        L = M + seg_len
        idx = jnp.arange(L)
        mask = (idx[:, None] < M) | (idx[:, None] >= idx[None, :])
        mem = mem0
        outs = []
        for s in range(n_seg):
            xs = x[:, s * seg_len:(s + 1) * seg_len, :].copy()
            h = jnp.concatenate([mem, xs], axis=1)
            q = jnp.einsum('btd,dhe->bhte', h, Wq)
            k = jnp.einsum('btd,dhe->bhte', h, Wk)
            v = jnp.einsum('btd,dhe->bhte', h, Wv)
            scores = jnp.einsum('bhqe,bhke->bhqk', q, k) * scale
            scores = jnp.where(mask[None, None], scores, -1000000000.0)
            p = _softmax(scores, axis=-1)
            o = jnp.einsum('bhqk,bhke->bhqe', p, v)
            o = jnp.einsum('bhte,hed->btd', o, Wo)
            mem = o[:, :M, :].copy()
            outs.append(o[:, M:, :])
        return jnp.concatenate(outs, axis=1)

    def _B_ref(x, wqkv, wo):
        B, S, D = x.shape
        H = 32
        Dh = D // H
        W, dil = (8, 2)
        qkv = (lambda x, *d: x.transpose(*d))((x @ wqkv).reshape(B, S, 3, H, Dh), 2, 0, 3, 1, 4)
        q, k, v = (qkv[0], qkv[1], qkv[2])
        scale = Dh ** (-0.5)
        pos = jnp.arange(S)
        off = jnp.arange(W) * dil
        idx = pos[:, None] - off[None, :]
        mask = idx >= 0
        idx_c = jnp.where(mask, idx, 0).reshape(-1)
        kg = k[:, :, idx_c, :].reshape(B, H, S, W, Dh)
        vg = v[:, :, idx_c, :].reshape(B, H, S, W, Dh)
        logits = jnp.einsum('bhsd,bhswd->bhsw', q, kg) * scale
        logits = jnp.where(mask[None, None, :, :], logits, -1000000000.0)
        attn = _softmax(logits, axis=-1)
        o = jnp.einsum('bhsw,bhswd->bhsd', attn, vg)
        return (lambda x, *d: x.transpose(*d))(o, 0, 2, 1, 3).reshape(B, S, D) @ wo
    x = A_x
    g = _sigmoid((x * gate_w).sum(-1, keepdims=True))
    a = _A_ref(x, A_mem0, A_Wq, A_Wk, A_Wv, A_Wo, A_seg_len)
    b = _B_ref(x, B_wqkv, B_wo)
    return g * a + (1 - g) * b
```

```python
import functools

import jax
import jax.numpy as jnp
from jax import lax
from jax.experimental import pallas as pl
from jax.experimental.pallas import tpu as pltpu

F32 = jnp.float32
BF16 = jnp.bfloat16
LANES = 128
NEG = -1000000000.0

B_HEADS = 32
B_WINDOW = 8
B_DIL = 2
B_HIST = 16
B_CHUNKS = 8


def _dot(a, b):
    return lax.dot_general(a, b, (((1,), (0,)), ((), ())), preferred_element_type=F32)


def _dot_nt(a, b):
    return lax.dot_general(a, b, (((1,), (1,)), ((), ())), preferred_element_type=F32)


def _kernel(x_hbm, mem0_ref, wq_hbm, wk_hbm, wv_hbm, wo_hbm, bqkv_hbm, bwo_hbm, gw_ref,
            out_hbm,
            x_v, raw_v, w_v, wo_v, bqkv_v, bwo_v, bqkv_p, bwo_p, q_s, k_s, v_s, ob_s, b_s,
            out_v, sem_in, sem_w, sem_out, *, seg, n_heads, dh):
    S, D = x_v.shape
    M = mem0_ref.shape[0]
    L = M + seg
    n_seg = S // seg
    n_pairs = n_heads // 2
    pw = 2 * dh
    nt = D // LANES
    T = S // B_CHUNKS
    ppc = n_pairs // B_CHUNKS
    slab = ppc * pw
    w_hbm = (wq_hbm, wk_hbm, wv_hbm)
    half = wo_v.shape[0] // 2

    cp_bqkv = pltpu.make_async_copy(bqkv_hbm, bqkv_v, sem_in.at[0])
    cp_x = pltpu.make_async_copy(x_hbm, x_v, sem_in.at[1])
    cp_bwo = pltpu.make_async_copy(bwo_hbm, bwo_v, sem_in.at[2])
    cp_wo = [pltpu.make_async_copy(wo_hbm.at[pl.ds(j * half, half)],
                                   wo_v.at[pl.ds(j * half, half)], sem_in.at[3 + j])
             for j in range(2)]

    def cp_w(j, c):
        r0 = pl.multiple_of(c * slab, slab)
        return pltpu.make_async_copy(w_hbm[j].at[pl.ds(r0, slab)],
                                     raw_v.at[j, pl.ds(r0, slab)], sem_w.at[j, c])

    cp_bqkv.start()
    cp_bwo.start()
    cp_x.start()

    bdh = D // B_HEADS
    src = lax.broadcasted_iota(jnp.int32, (D, D), 0)
    dst = lax.broadcasted_iota(jnp.int32, (D, D), 1)
    perm = (src == (dst % B_HEADS) * bdh + dst // B_HEADS).astype(BF16)
    perm_t = (dst == (src % B_HEADS) * bdh + src // B_HEADS).astype(BF16)
    cp_bqkv.wait()
    for j in range(3):
        cp_w(j, 0).start()
    for j in range(3):
        cs = slice(j * D, (j + 1) * D)
        bqkv_p[:, cs] = _dot(bqkv_v[:, cs], perm).astype(BF16)
    cp_bwo.wait()
    bwo_p[...] = _dot(perm_t, bwo_v[...]).astype(BF16)
    cp_x.wait()
    for j in range(3):
        cp_w(j, 1).start()

    b_scale = bdh ** -0.5

    def b_chunk(c, carry):
        for j in range(3):
            cp_w(j, c).wait()

        @pl.when(c + 2 < B_CHUNKS)
        def _():
            for j in range(3):
                cp_w(j, c + 2).start()

        for j in range(2):
            @pl.when(c + 2 == B_CHUNKS + j)
            def _():
                cp_wo[j].start()

        r0 = pl.multiple_of(c * T, T)
        xc = x_v[pl.ds(r0, T), :]
        kk = _dot(xc, bqkv_p[:, D:2 * D])
        vv = _dot(xc, bqkv_p[:, 2 * D:3 * D])
        first = c == 0
        for t in range(nt):
            ls = slice(t * LANES, (t + 1) * LANES)
            k0 = jnp.broadcast_to(kk[0:1, ls], (B_HIST, LANES))
            v0 = jnp.broadcast_to(vv[0:1, ls], (B_HIST, LANES))
            k_s[t, 0:B_HIST, :] = jnp.where(first, k0, k_s[t, T:T + B_HIST, :])
            v_s[t, 0:B_HIST, :] = jnp.where(first, v0, v_s[t, T:T + B_HIST, :])
            k_s[t, B_HIST:B_HIST + T, :] = kk[:, ls]
            v_s[t, B_HIST:B_HIST + T, :] = vv[:, ls]
        q_s[...] = _dot(xc, bqkv_p[:, 0:D])

        for j in range(3):
            for u in range(ppc):
                p = c * ppc + u
                rr = pl.multiple_of(p * pw, pw)
                w_v[p, :, j * pw:(j + 1) * pw] = raw_v[j, pl.ds(rr, pw), :].T

        G = 32
        for g in range(T // G):
            g0 = g * G
            qs = [q_s[g0:g0 + G, t * LANES:(t + 1) * LANES] for t in range(nt)]
            pos = r0 + g0 + lax.broadcasted_iota(jnp.int32, (G, LANES), 0)
            logits = []
            for w in range(B_WINDOW):
                o0 = B_HIST + g0 - w * B_DIL
                acc = qs[0] * k_s[0, o0:o0 + G, :]
                for t in range(1, nt):
                    acc = acc + qs[t] * k_s[t, o0:o0 + G, :]
                sh = LANES // 2
                while sh >= B_HEADS:
                    acc = acc + pltpu.roll(acc, sh, 1)
                    sh //= 2
                acc = acc * b_scale
                if g0 < w * B_DIL:
                    acc = jnp.where(pos >= w * B_DIL, acc, NEG)
                logits.append(acc)
            mx = functools.reduce(jnp.maximum, logits)
            es = [jnp.exp(l - mx) for l in logits]
            inv = 1.0 / functools.reduce(jnp.add, es)
            ps = [e * inv for e in es]
            for t in range(nt):
                acc = None
                for w in range(B_WINDOW):
                    o0 = B_HIST + g0 - w * B_DIL
                    term = ps[w] * v_s[t, o0:o0 + G, :]
                    acc = term if acc is None else acc + term
                ob_s[g0:g0 + G, t * LANES:(t + 1) * LANES] = acc.astype(BF16)
        b_s[pl.ds(r0, T), :] = _dot(ob_s[...], bwo_p[...])
        return carry

    for t in range(nt):
        k_s[t, T:T + B_HIST, :] = jnp.zeros((B_HIST, LANES), F32)
        v_s[t, T:T + B_HIST, :] = jnp.zeros((B_HIST, LANES), F32)
    lax.fori_loop(0, B_CHUNKS, b_chunk, 0)
    for j in range(2):
        cp_wo[j].wait()

    a_scale = dh ** -0.5
    gw = gw_ref[...].astype(F32)

    def cp_out(s):
        r0 = pl.multiple_of(s * seg, seg)
        return pltpu.make_async_copy(out_v.at[pl.ds(r0, seg)], out_hbm.at[pl.ds(r0, seg)],
                                     sem_out.at[0])

    def split_pair(z):
        col = lax.broadcasted_iota(jnp.int32, z.shape, 1)
        return jnp.concatenate([jnp.where(col < dh, z, 0.0), jnp.where(col >= dh, z, 0.0)],
                               axis=0).astype(BF16)

    def step(s, mem):
        r0 = pl.multiple_of(s * seg, seg)
        xs = x_v[pl.ds(r0, seg), :].astype(F32)
        h = jnp.concatenate([mem, xs], axis=0)
        row = lax.broadcasted_iota(jnp.int32, (L, 2 * L), 0)
        col = lax.broadcasted_iota(jnp.int32, (L, 2 * L), 1)
        in_a = col < L
        visible = (row < M) | (row >= jnp.where(in_a, col, col - L))

        def proj(p):
            return _dot(h, w_v[p])

        def scores(qkv):
            return _dot_nt(qkv[:, 0:pw], split_pair(qkv[:, pw:2 * pw]))

        def attend(qkv, sc):
            sc = jnp.where(visible, sc * a_scale, NEG)
            ma = jnp.max(jnp.where(in_a, sc, -jnp.inf), axis=1, keepdims=True)
            mb = jnp.max(jnp.where(in_a, -jnp.inf, sc), axis=1, keepdims=True)
            e = jnp.exp(sc - jnp.where(in_a, ma, mb))
            la = jnp.sum(jnp.where(in_a, e, 0.0), axis=1, keepdims=True)
            lb = jnp.sum(jnp.where(in_a, 0.0, e), axis=1, keepdims=True)
            pr = e * jnp.where(in_a, 1.0 / la, 1.0 / lb)
            return _dot(pr, split_pair(qkv[:, 2 * pw:3 * pw]))

        qkv, sc, o = {}, {}, {}
        acc = None
        for i in range(n_pairs + 3):
            if i < n_pairs:
                qkv[i] = proj(i)
            if 0 <= i - 1 < n_pairs:
                sc[i - 1] = scores(qkv[i - 1])
            if 0 <= i - 2 < n_pairs:
                o[i - 2] = attend(qkv.pop(i - 2), sc.pop(i - 2))
            if 0 <= i - 3 < n_pairs:
                p = i - 3
                term = _dot(o.pop(p), wo_v[p * pw:(p + 1) * pw, :])
                acc = term if acc is None else acc + term

        g = jax.nn.sigmoid(jnp.sum(xs * gw, axis=1, keepdims=True))
        res = g * acc[M:, :] + (1.0 - g) * b_s[pl.ds(r0, seg), :]
        out_v[pl.ds(r0, seg), :] = res.astype(out_v.dtype)
        cp_out(s).start()
        return acc[:M, :].astype(BF16).astype(F32)

    lax.fori_loop(0, n_seg, step, mem0_ref[...].astype(F32))
    pltpu.make_async_copy(out_v, out_hbm, sem_out.at[0]).wait()


@functools.partial(jax.jit, static_argnames=("A_seg_len",))
def pallas_gated_mix__memory_aug_recurrent_mem_tr__sliding_local_dilated__prompt_kernel(
    A_x, A_mem0, A_Wq, A_Wk, A_Wv, A_Wo, A_seg_len, B_x, B_wqkv, B_wo, gate_w,
):
    del B_x
    _, S, D = A_x.shape
    _, H, Dh = A_Wq.shape
    M = A_mem0.shape[1]
    seg = int(A_seg_len)
    HD = H * Dh
    T = S // B_CHUNKS
    nt = D // LANES

    def rows(w):
        return jnp.transpose(w, (1, 2, 0)).reshape(HD, D)

    hbm = pl.BlockSpec(memory_space=pl.ANY)
    vmem = pl.BlockSpec(memory_space=pltpu.VMEM)
    out = pl.pallas_call(
        functools.partial(_kernel, seg=seg, n_heads=H, dh=Dh),
        out_shape=jax.ShapeDtypeStruct((S, D), A_x.dtype),
        in_specs=[hbm, vmem, hbm, hbm, hbm, hbm, hbm, hbm, vmem],
        out_specs=hbm,
        scratch_shapes=[
            pltpu.VMEM((S, D), BF16),
            pltpu.VMEM((3, HD, D), BF16),
            pltpu.VMEM((H // 2, D, 6 * Dh), BF16),
            pltpu.VMEM((HD, D), BF16),
            pltpu.VMEM((D, 3 * D), BF16),
            pltpu.VMEM((D, D), BF16),
            pltpu.VMEM((D, 3 * D), BF16),
            pltpu.VMEM((D, D), BF16),
            pltpu.VMEM((T, D), F32),
            pltpu.VMEM((nt, B_HIST + T, LANES), F32),
            pltpu.VMEM((nt, B_HIST + T, LANES), F32),
            pltpu.VMEM((T, D), BF16),
            pltpu.VMEM((S, D), F32),
            pltpu.VMEM((S, D), A_x.dtype),
            pltpu.SemaphoreType.DMA((5,)),
            pltpu.SemaphoreType.DMA((3, B_CHUNKS)),
            pltpu.SemaphoreType.DMA((1,)),
        ],
        compiler_params=pltpu.CompilerParams(vmem_limit_bytes=110 * 2**20),
    )(A_x.reshape(S, D), A_mem0.reshape(M, D), rows(A_Wq), rows(A_Wk), rows(A_Wv),
      A_Wo.reshape(HD, D), B_wqkv, B_wo, gate_w.reshape(1, D))
    return out.reshape(A_x.shape)
```

```python
import functools

import jax
import jax.numpy as jnp
from jax import lax
from jax.experimental import pallas as pl
from jax.experimental.pallas import tpu as pltpu

F32 = jnp.float32
BF16 = jnp.bfloat16
LANES = 128
NEG = -1000000000.0

B_HEADS = 32
B_WINDOW = 8
B_DIL = 2
B_HIST = 16
B_GROUP = 32

CHUNKS = 8
SUB = 64
SUBS = 4
UNROLL = 3
LAG_SCORES, LAG_ATTEND, LAG_OUT = 1, 3, 5


def _dot(a, b):
    return lax.dot_general(a, b, (((1,), (0,)), ((), ())), preferred_element_type=F32)


def _dot_nt(a, b):
    return lax.dot_general(a, b, (((1,), (1,)), ((), ())), preferred_element_type=F32)


def _pack(a):
    return pltpu.bitcast(a, jnp.uint32)


def _unpack(a):
    return pltpu.bitcast(a, BF16)


def _kernel(x_hbm, mem0_hbm, wq_hbm, wk_hbm, wv_hbm, wo_hbm, bqkv_hbm, bwo_hbm, gw_hbm,
            out_hbm,
            mem0_ref, gw_ref, x_v, raw_v, w_v, wo_v, bqkv_v, bwo_v, perm_s, bqkv_p, bwo_p, q_s, k_s, v_s, ob_s,
            b_s, acc_s, out_v, sem_b, sem_w, sem_out, *, seg, n_heads, dh):
    S, D = x_v.shape
    M = mem0_ref.shape[0]
    L = M + seg
    n_seg = S // seg
    n_pairs = n_heads // 2
    pw = 2 * dh
    nt = D // LANES
    T = S // CHUNKS
    ppc = n_pairs // CHUNKS
    slab = ppc * pw
    w_hbm = (wq_hbm, wk_hbm, wv_hbm, wo_hbm)
    bdh = D // B_HEADS
    b_scale = bdh ** -0.5
    a_scale = dh ** -0.5

    def aligned(i, n):
        return i * n if isinstance(i, int) else pl.multiple_of(i * n, n)

    cp_bqkv = pltpu.make_async_copy(bqkv_hbm, bqkv_v, sem_b.at[0])
    cp_bwo = pltpu.make_async_copy(bwo_hbm, bwo_v, sem_b.at[1])

    cp_small = [pltpu.make_async_copy(mem0_hbm, mem0_ref, sem_b.at[2]),
                pltpu.make_async_copy(gw_hbm, gw_ref, sem_b.at[3])]

    def cp_x(c):
        rows = pl.ds(aligned(c, T), T)
        return pltpu.make_async_copy(x_hbm.at[rows], x_v.at[rows], sem_w.at[4 * CHUNKS + c])

    def cp_w(c):
        rows = pl.ds(aligned(c, slab), slab)
        return [pltpu.make_async_copy(w_hbm[j].at[rows], raw_v.at[j, rows],
                                      sem_w.at[j * CHUNKS + c]) for j in range(4)]

    def cp_out(s, n):
        rows = pl.ds(aligned(s, seg), n * seg)
        return pltpu.make_async_copy(out_v.at[rows], out_hbm.at[rows], sem_out.at[0])

    def start(copies):
        for cp in copies:
            cp.start()

    def wait(copies):
        for cp in copies:
            cp.wait()

    def reorder_rows(w, dst_ref, r0):
        wf = w.astype(F32)
        for t in range(nt):
            perm_s[t] = wf[:, t * LANES:(t + 1) * LANES]
        for d in range(bdh):
            blk = [perm_s[t, pl.ds(d, B_HEADS, stride=bdh), :] for t in range(nt)]
            o0 = (r0 + d * B_HEADS) // 2
            dst_ref[o0:o0 + B_HEADS // 2, :] = _pack(jnp.concatenate(blk, axis=1).astype(BF16))

    def b_project(c, u, is_first):
        rows = pl.ds(aligned(c * SUBS + u, SUB), SUB)
        xc = x_v[rows, :]
        o0 = B_HIST + u * SUB
        for ref, j in ((k_s, 1), (v_s, 2)):
            z = _dot_nt(xc, _unpack(bqkv_p[j * D // 2:(j + 1) * D // 2, :]))
            for t in range(nt):
                zt = z[:, t * LANES:(t + 1) * LANES]
                if u == 0 and is_first:
                    ref[t, 0:B_HIST, :] = jnp.broadcast_to(zt[0:1, :], (B_HIST, LANES))
                elif u == 0:
                    ref[t, 0:B_HIST, :] = ref[t, T:T + B_HIST, :]
                ref[t, o0:o0 + SUB, :] = zt
        q_s[u * SUB:(u + 1) * SUB, :] = _dot_nt(xc, _unpack(bqkv_p[0:D // 2, :]))

    def b_attend(u, is_first):
        G = B_GROUP
        for g0 in range(u * SUB, (u + 1) * SUB, G):
            qs = [q_s[g0:g0 + G, t * LANES:(t + 1) * LANES] for t in range(nt)]
            logits = []
            for w in range(B_WINDOW):
                o0 = B_HIST + g0 - w * B_DIL
                acc = qs[0] * k_s[0, o0:o0 + G, :]
                for t in range(1, nt):
                    acc = acc + qs[t] * k_s[t, o0:o0 + G, :]
                sh = LANES // 2
                while sh >= B_HEADS:
                    acc = acc + pltpu.roll(acc, sh, 1)
                    sh //= 2
                acc = acc * b_scale
                if is_first and g0 < w * B_DIL:
                    pos = g0 + lax.broadcasted_iota(jnp.int32, (G, LANES), 0)
                    acc = jnp.where(pos >= w * B_DIL, acc, NEG)
                logits.append(acc)
            mx = functools.reduce(jnp.maximum, logits)
            es = [jnp.exp(l - mx) for l in logits]
            inv = 1.0 / functools.reduce(jnp.add, es)
            ps = [e * inv for e in es]
            for t in range(nt):
                acc = None
                for w in range(B_WINDOW):
                    o0 = B_HIST + g0 - w * B_DIL
                    term = ps[w] * v_s[t, o0:o0 + G, :]
                    acc = term if acc is None else acc + term
                ob_s[g0:g0 + G, t * LANES:(t + 1) * LANES] = acc.astype(BF16)

    def b_output(c, u):
        rows = pl.ds(aligned(c * SUBS + u, SUB), SUB)
        b_s[rows, :] = _dot(ob_s[u * SUB:(u + 1) * SUB, :], _unpack(bwo_p[...]))

    def relayout(c):
        for u in range(ppc):
            p = c * ppc + u
            rows = pl.ds(aligned(p, pw), pw)
            for j in range(3):
                w_v[p, :, j * pw:(j + 1) * pw] = _pack(raw_v[j, rows, :].T)
            wo_v[p] = _pack(raw_v[3, rows, :])

    def split_pair(z):
        col = lax.broadcasted_iota(jnp.int32, z.shape, 1)
        return jnp.concatenate([jnp.where(col < dh, z, 0.0), jnp.where(col >= dh, z, 0.0)],
                               axis=0).astype(BF16)

    def a_project(h, p):
        return _dot(h, _unpack(w_v[p]))

    def a_scores(qkv):
        return _dot_nt(qkv[:, 0:pw], split_pair(qkv[:, pw:2 * pw]))

    def a_attend(qkv, sc):
        row = lax.broadcasted_iota(jnp.int32, (L, 2 * L), 0)
        col = lax.broadcasted_iota(jnp.int32, (L, 2 * L), 1)
        in_a = col < L
        visible = (row < M) | (row >= jnp.where(in_a, col, col - L))
        sc = jnp.where(visible, sc * a_scale, NEG)
        ma = jnp.max(jnp.where(in_a, sc, -jnp.inf), axis=1, keepdims=True)
        mb = jnp.max(jnp.where(in_a, -jnp.inf, sc), axis=1, keepdims=True)
        e = jnp.exp(sc - jnp.where(in_a, ma, mb))
        la = jnp.sum(jnp.where(in_a, e, 0.0), axis=1, keepdims=True)
        lb = jnp.sum(jnp.where(in_a, 0.0, e), axis=1, keepdims=True)
        pr = e * (1.0 / jnp.where(in_a, la, lb))
        return _dot(pr, split_pair(qkv[:, 2 * pw:3 * pw]))

    def a_output(o, p):
        return _dot(o, _unpack(wo_v[p]))

    def a_tokens(s, mem):
        xs = x_v[pl.ds(aligned(s, seg), seg), :].astype(F32)
        return jnp.concatenate([mem, xs], axis=0)

    def finish(s, acc):
        rows = pl.ds(aligned(s, seg), seg)
        xs = x_v[rows, :].astype(F32)
        g = jax.nn.sigmoid(jnp.sum(xs * gw_ref[...].astype(F32), axis=1, keepdims=True))
        out_v[rows, :] = (g * acc[M:, :] + (1.0 - g) * b_s[rows, :]).astype(out_v.dtype)
        return acc[:M, :].astype(BF16).astype(F32)

    def warmup(cb, ca):
        first = ca is None
        nb = 0 if cb is None else SUBS
        pairs = [] if ca is None else [ca * ppc + u for u in range(ppc)]
        if pairs:
            relayout(ca)
            h = a_tokens(0, mem0_ref[...].astype(F32))
        qkv, sc, o = {}, {}, {}
        for u in range(nb):
            b_project(cb, u, first)
            if u + 1 < nb:
                b_attend(u, first)
        if pairs:
            qkv[0] = a_project(h, pairs[0])
        if nb:
            b_attend(nb - 1, first)
        if pairs:
            qkv[1] = a_project(h, pairs[1])
            sc[0] = a_scores(qkv[0])
            sc[1] = a_scores(qkv[1])
        for u in range(nb // 2):
            b_output(cb, u)
        if pairs:
            o[0] = a_attend(qkv[0], sc[0])
            o[1] = a_attend(qkv[1], sc[1])
        for u in range(nb // 2, nb):
            b_output(cb, u)
        if pairs:
            acc_s[...] += a_output(o[0], pairs[0]) + a_output(o[1], pairs[1])

    cp_bqkv.start()
    cp_x(0).start()
    cp_bwo.start()
    start(cp_small)
    acc_s[...] = jnp.zeros(acc_s.shape, F32)
    cp_bqkv.wait()
    cp_x(1).start()
    start(cp_w(0))
    for j in range(3):
        reorder_rows(bqkv_v[:, j * D:(j + 1) * D].T, bqkv_p, j * D)
    cp_bwo.wait()
    reorder_rows(bwo_v[...], bwo_p, 0)
    cp_x(0).wait()
    wait(cp_small)
    cp_x(2).start()
    start(cp_w(1))
    warmup(0, None)

    def warmup_step(c, carry):
        cp_x(c).wait()
        wait(cp_w(c - 1))

        @pl.when(c + 2 < CHUNKS)
        def _():
            cp_x(c + 2).start()

        @pl.when(c + 1 < CHUNKS)
        def _():
            start(cp_w(c + 1))

        warmup(c, c - 1)
        return carry

    lax.fori_loop(1, CHUNKS, warmup_step, 0)
    wait(cp_w(CHUNKS - 1))
    warmup(None, CHUNKS - 1)
    mem1 = finish(0, acc_s[...])
    cp_out(0, 1).start()

    def step(s, mem):
        h = a_tokens(s, mem)
        qkv, sc, o = {}, {}, {}
        acc = None
        for i in range(n_pairs + LAG_OUT):
            if i < n_pairs:
                qkv[i] = a_project(h, i)
            p = i - LAG_SCORES
            if 0 <= p < n_pairs:
                sc[p] = a_scores(qkv[p])
            p = i - LAG_OUT
            if 0 <= p < n_pairs:
                term = a_output(o.pop(p), p)
                acc = term if acc is None else acc + term
            p = i - LAG_ATTEND
            if 0 <= p < n_pairs:
                o[p] = a_attend(qkv.pop(p), sc.pop(p))
        return finish(s, acc)

    def steps(i, mem):
        s0 = 1 + i * UNROLL
        for u in range(UNROLL):
            mem = step(s0 + u, mem)
        cp_out(s0, UNROLL).start()
        return mem

    assert (n_seg - 1) % UNROLL == 0
    lax.fori_loop(0, (n_seg - 1) // UNROLL, steps, mem1)
    pltpu.make_async_copy(out_v, out_hbm, sem_out.at[0]).wait()


@functools.partial(jax.jit, static_argnames=("A_seg_len",))
def pallas_gated_mix__memory_aug_recurrent_mem_tr__sliding_local_dilated__prompt_kernel(
    A_x, A_mem0, A_Wq, A_Wk, A_Wv, A_Wo, A_seg_len, B_x, B_wqkv, B_wo, gate_w,
):
    del B_x
    _, S, D = A_x.shape
    _, H, Dh = A_Wq.shape
    M = A_mem0.shape[1]
    seg = int(A_seg_len)
    HD = H * Dh
    T = S // CHUNKS
    assert T == SUB * SUBS and H == 4 * CHUNKS
    nt = D // LANES

    def rows(w):
        return jnp.transpose(w, (1, 2, 0)).reshape(HD, D)

    hbm = pl.BlockSpec(memory_space=pl.ANY)
    out = pl.pallas_call(
        functools.partial(_kernel, seg=seg, n_heads=H, dh=Dh),
        out_shape=jax.ShapeDtypeStruct((S, D), A_x.dtype),
        in_specs=[hbm] * 9,
        out_specs=hbm,
        scratch_shapes=[
            pltpu.VMEM((M, D), BF16),
            pltpu.VMEM((1, D), BF16),
            pltpu.VMEM((S, D), BF16),
            pltpu.VMEM((4, HD, D), BF16),
            pltpu.VMEM((H // 2, D // 2, 6 * Dh), jnp.uint32),
            pltpu.VMEM((H // 2, Dh, D), jnp.uint32),
            pltpu.VMEM((D, 3 * D), BF16),
            pltpu.VMEM((D, D), BF16),
            pltpu.VMEM((nt, D, LANES), F32),
            pltpu.VMEM((3 * D // 2, D), jnp.uint32),
            pltpu.VMEM((D // 2, D), jnp.uint32),
            pltpu.VMEM((T, D), F32),
            pltpu.VMEM((nt, B_HIST + T, LANES), F32),
            pltpu.VMEM((nt, B_HIST + T, LANES), F32),
            pltpu.VMEM((T, D), BF16),
            pltpu.VMEM((S, D), F32),
            pltpu.VMEM((M + seg, D), F32),
            pltpu.VMEM((S, D), A_x.dtype),
            pltpu.SemaphoreType.DMA((4,)),
            pltpu.SemaphoreType.DMA((5 * CHUNKS,)),
            pltpu.SemaphoreType.DMA((1,)),
        ],
        compiler_params=pltpu.CompilerParams(vmem_limit_bytes=110 * 2**20),
    )(A_x.reshape(S, D), A_mem0.reshape(M, D), rows(A_Wq), rows(A_Wk), rows(A_Wv),
      A_Wo.reshape(HD, D), B_wqkv, B_wo, gate_w.reshape(1, D))
    return out.reshape(A_x.shape)
```

```python
import functools

import jax
import jax.numpy as jnp
from jax import lax
from jax.experimental import pallas as pl
from jax.experimental.pallas import tpu as pltpu

F32 = jnp.float32
BF16 = jnp.bfloat16
LANES = 128
NEG = -1000000000.0
LOG2E = 1.4426950408889634

B_HEADS = 32
B_WINDOW = 8
B_DIL = 2
B_HIST = 16
B_GROUP = 32

CHUNKS = 8
SUB = 128
SUBS = 2
UNROLL = 3
LAG_SCORES, LAG_ATTEND, LAG_OUT = 1, 3, 5


def _dot(a, b):
    return lax.dot_general(a, b, (((1,), (0,)), ((), ())), preferred_element_type=F32)


def _dot_nt(a, b):
    return lax.dot_general(a, b, (((1,), (1,)), ((), ())), preferred_element_type=F32)


def _pack(a):
    return pltpu.bitcast(a, jnp.uint32)


def _unpack(a):
    return pltpu.bitcast(a, BF16)


def _kernel(x_hbm, mem0_hbm, wq_hbm, wk_hbm, wv_hbm, wo_hbm, bqkv_hbm, bwo_hbm, gw_hbm,
            out_hbm,
            mem0_ref, gw_ref, x_v, raw_v, w_v, wo_v, bqkv_v, bwo_v, perm_s, bqkv_p, bwo_p, q_s, k_s, v_s, ob_s,
            b_s, acc_s, out_v, sem_b, sem_w, sem_out, *, seg, n_heads, dh):
    S, D = x_v.shape
    M = mem0_ref.shape[0]
    L = M + seg
    n_seg = S // seg
    n_pairs = n_heads // 2
    pw = 2 * dh
    nt = D // LANES
    T = S // CHUNKS
    ppc = n_pairs // CHUNKS
    slab = ppc * pw
    w_hbm = (wq_hbm, wk_hbm, wv_hbm, wo_hbm)
    bdh = D // B_HEADS
    b_scale = bdh ** -0.5
    a_scale = dh ** -0.5

    def aligned(i, n):
        return i * n if isinstance(i, int) else pl.multiple_of(i * n, n)

    cp_bqkv = [pltpu.make_async_copy(bqkv_hbm.at[:, pl.ds(j * D, D)], bqkv_v.at[j],
                                     sem_b.at[4 + j]) for j in range(3)]
    cp_bwo = pltpu.make_async_copy(bwo_hbm, bwo_v, sem_b.at[1])

    cp_small = [pltpu.make_async_copy(mem0_hbm, mem0_ref, sem_b.at[2]),
                pltpu.make_async_copy(gw_hbm, gw_ref, sem_b.at[3])]

    def cp_x(c):
        rows = pl.ds(aligned(c, T), T)
        return pltpu.make_async_copy(x_hbm.at[rows], x_v.at[rows], sem_w.at[4 * CHUNKS + c])

    def cp_w(c):
        rows = pl.ds(aligned(c, slab), slab)
        return [pltpu.make_async_copy(w_hbm[j].at[rows], raw_v.at[j, rows],
                                      sem_w.at[j * CHUNKS + c]) for j in range(4)]

    def cp_out(s, n):
        rows = pl.ds(aligned(s, seg), n * seg)
        return pltpu.make_async_copy(out_v.at[rows], out_hbm.at[rows], sem_out.at[0])

    def start(copies):
        for cp in copies:
            cp.start()

    def wait(copies):
        for cp in copies:
            cp.wait()

    def reorder_rows(w, dst_ref, r0):
        wf = w.astype(F32)
        for t in range(nt):
            perm_s[t] = wf[:, t * LANES:(t + 1) * LANES]
        for d in range(bdh):
            blk = [perm_s[t, pl.ds(d, B_HEADS, stride=bdh), :] for t in range(nt)]
            o0 = (r0 + d * B_HEADS) // 2
            dst_ref[o0:o0 + B_HEADS // 2, :] = _pack(jnp.concatenate(blk, axis=1).astype(BF16))

    def b_project(c, u, j, is_first):
        xc = x_v[pl.ds(aligned(c * SUBS + u, SUB), SUB), :]
        z = _dot_nt(xc, _unpack(bqkv_p[j * D // 2:(j + 1) * D // 2, :]))
        if j == 0:
            q_s[u * SUB:(u + 1) * SUB, :] = z
            return
        ref = k_s if j == 1 else v_s
        o0 = B_HIST + u * SUB
        for t in range(nt):
            zt = z[:, t * LANES:(t + 1) * LANES]
            if u == 0 and is_first:
                ref[t, 0:B_HIST, :] = jnp.broadcast_to(zt[0:1, :], (B_HIST, LANES))
            elif u == 0:
                ref[t, 0:B_HIST, :] = ref[t, T:T + B_HIST, :]
            ref[t, o0:o0 + SUB, :] = zt

    def b_attend(g0, is_first):
        G = B_GROUP

        def windows(ref, t):
            views = {}
            for r in range(0, 8, B_DIL):
                shifts = range(r, B_WINDOW * B_DIL, 8)
                back = shifts[-1]
                o0 = B_HIST + g0 - back
                z = ref[t, o0:o0 + G + back - r, :]
                for sft in shifts:
                    views[sft // B_DIL] = z[back - sft:back - sft + G, :]
            return views

        logits = [None] * B_WINDOW
        for t in range(nt):
            qt = q_s[g0:g0 + G, t * LANES:(t + 1) * LANES]
            for w, kw in windows(k_s, t).items():
                logits[w] = qt * kw if t == 0 else logits[w] + qt * kw
        for w in range(B_WINDOW):
            acc = logits[w]
            sh = LANES // 2
            while sh >= B_HEADS:
                acc = acc + pltpu.roll(acc, sh, 1)
                sh //= 2
            if is_first and g0 < w * B_DIL:
                pos = g0 + lax.broadcasted_iota(jnp.int32, (G, LANES), 0)
                acc = jnp.where(pos >= w * B_DIL, acc, NEG / b_scale)
            logits[w] = acc
        mx = functools.reduce(jnp.maximum, logits)
        es = [jnp.exp2((l - mx) * (b_scale * LOG2E)) for l in logits]
        inv = 1.0 / functools.reduce(jnp.add, es)
        for t in range(nt):
            terms = [es[w] * vw for w, vw in windows(v_s, t).items()]
            acc = functools.reduce(jnp.add, terms) * inv
            ob_s[g0:g0 + G, t * LANES:(t + 1) * LANES] = acc.astype(BF16)

    def b_output(c, u):
        rows = pl.ds(aligned(c * SUBS + u, SUB), SUB)
        b_s[rows, :] = _dot(ob_s[u * SUB:(u + 1) * SUB, :], _unpack(bwo_p[...]))

    def relayout(c):
        for u in range(ppc):
            p = c * ppc + u
            rows = pl.ds(aligned(p, pw), pw)
            for j in range(3):
                w_v[p, :, j * pw:(j + 1) * pw] = _pack(raw_v[j, rows, :].T)
            wo_v[p] = _pack(raw_v[3, rows, :])

    def split_pair(z):
        col = lax.broadcasted_iota(jnp.int32, z.shape, 1)
        return jnp.concatenate([jnp.where(col < dh, z, 0.0), jnp.where(col >= dh, z, 0.0)],
                               axis=0).astype(BF16)

    def a_project(h, p):
        return _dot(h, _unpack(w_v[p]))

    def a_scores(qkv):
        return _dot_nt(qkv[:, 0:pw], split_pair(qkv[:, pw:2 * pw]))

    def a_attend(qkv, sc):
        row = lax.broadcasted_iota(jnp.int32, (L, 2 * L), 0)
        col = lax.broadcasted_iota(jnp.int32, (L, 2 * L), 1)
        in_a = col < L
        visible = (row < M) | (row >= jnp.where(in_a, col, col - L))
        sc = jnp.where(visible, sc * a_scale, NEG)
        ma = jnp.max(jnp.where(in_a, sc, -jnp.inf), axis=1, keepdims=True)
        mb = jnp.max(jnp.where(in_a, -jnp.inf, sc), axis=1, keepdims=True)
        e = jnp.exp(sc - jnp.where(in_a, ma, mb))
        la = jnp.sum(jnp.where(in_a, e, 0.0), axis=1, keepdims=True)
        lb = jnp.sum(jnp.where(in_a, 0.0, e), axis=1, keepdims=True)
        pr = e * (1.0 / jnp.where(in_a, la, lb))
        return _dot(pr, split_pair(qkv[:, 2 * pw:3 * pw]))

    def a_output(o, p):
        return _dot(o, _unpack(wo_v[p]))

    def a_tokens(s, mem):
        xs = x_v[pl.ds(aligned(s, seg), seg), :].astype(F32)
        return jnp.concatenate([mem, xs], axis=0)

    def finish(s, acc):
        rows = pl.ds(aligned(s, seg), seg)
        xs = x_v[rows, :].astype(F32)
        g = jax.nn.sigmoid(jnp.sum(xs * gw_ref[...].astype(F32).reshape(1, D), axis=1, keepdims=True))
        out_v[rows, :] = (g * acc[M:, :] + (1.0 - g) * b_s[rows, :]).astype(out_v.dtype)
        return acc[:M, :]

    def warmup(cb, ca):
        first = ca is None
        nb = 0 if cb is None else SUBS
        pairs = [] if ca is None else [ca * ppc + u for u in range(ppc)]
        if pairs:
            relayout(ca)
            h = a_tokens(0, mem0_ref[...].astype(F32))
        qkv, sc, o = {}, {}, {}
        pending = []

        def drain(n):
            for _ in range(min(n, len(pending))):
                b_attend(pending.pop(0), first)

        gps = SUB // B_GROUP
        for u in range(nb):
            for n, j in enumerate((1, 2, 0)):
                b_project(cb, u, j, first)
                drain(gps * (n + 1) // 3 - gps * n // 3)
            pending.extend(range(u * SUB, (u + 1) * SUB, B_GROUP))
        if pairs:
            qkv[0] = a_project(h, pairs[0])
            drain(gps // 2)
            qkv[1] = a_project(h, pairs[1])
            drain(gps)
            sc[0] = a_scores(qkv[0])
            sc[1] = a_scores(qkv[1])
        for u in range(nb // 2):
            b_output(cb, u)
            drain(-(-gps // (nb // 2)))
        if pairs:
            o[0] = a_attend(qkv[0], sc[0])
            o[1] = a_attend(qkv[1], sc[1])
        for u in range(nb // 2, nb):
            b_output(cb, u)
        if pairs:
            acc_s[...] += a_output(o[0], pairs[0]) + a_output(o[1], pairs[1])

    cp_bqkv[0].start()
    cp_bqkv[1].start()
    start(cp_small)
    acc_s[...] = jnp.zeros(acc_s.shape, F32)
    cp_bqkv[0].wait()
    cp_bqkv[2].start()
    cp_x(0).start()
    reorder_rows(bqkv_v[0].T, bqkv_p, 0)
    cp_bqkv[1].wait()
    cp_bwo.start()
    cp_x(1).start()
    reorder_rows(bqkv_v[1].T, bqkv_p, D)
    cp_bqkv[2].wait()
    start(cp_w(0))
    reorder_rows(bqkv_v[2].T, bqkv_p, 2 * D)
    cp_bwo.wait()
    cp_x(0).wait()
    wait(cp_small)
    cp_x(2).start()
    start(cp_w(1))
    reorder_rows(bwo_v[...], bwo_p, 0)
    warmup(0, None)

    def warmup_step(c, carry):
        cp_x(c).wait()
        wait(cp_w(c - 1))

        @pl.when(c + 2 < CHUNKS)
        def _():
            cp_x(c + 2).start()

        @pl.when(c + 1 < CHUNKS)
        def _():
            start(cp_w(c + 1))

        warmup(c, c - 1)
        return carry

    lax.fori_loop(1, CHUNKS, warmup_step, 0)
    wait(cp_w(CHUNKS - 1))
    warmup(None, CHUNKS - 1)
    mem1 = finish(0, acc_s[...])
    cp_out(0, 1).start()

    def step(s, mem):
        h = a_tokens(s, mem)
        qkv, sc, o = {}, {}, {}
        acc = None
        for i in range(n_pairs + LAG_OUT):
            if i < n_pairs:
                qkv[i] = a_project(h, i)
            p = i - LAG_SCORES
            if 0 <= p < n_pairs:
                sc[p] = a_scores(qkv[p])
            p = i - LAG_OUT
            if 0 <= p < n_pairs:
                term = a_output(o.pop(p), p)
                acc = term if acc is None else acc + term
            p = i - LAG_ATTEND
            if 0 <= p < n_pairs:
                o[p] = a_attend(qkv.pop(p), sc.pop(p))
        return finish(s, acc)

    def steps(i, mem):
        s0 = 1 + i * UNROLL
        for u in range(UNROLL):
            mem = step(s0 + u, mem)
        cp_out(s0, UNROLL).start()
        return mem

    assert (n_seg - 1) % UNROLL == 0
    lax.fori_loop(0, (n_seg - 1) // UNROLL, steps, mem1)
    pltpu.make_async_copy(out_v, out_hbm, sem_out.at[0]).wait()


@functools.partial(jax.jit, static_argnames=("A_seg_len",))
def pallas_gated_mix__memory_aug_recurrent_mem_tr__sliding_local_dilated__prompt_kernel(
    A_x, A_mem0, A_Wq, A_Wk, A_Wv, A_Wo, A_seg_len, B_x, B_wqkv, B_wo, gate_w,
):
    del B_x
    _, S, D = A_x.shape
    _, H, Dh = A_Wq.shape
    M = A_mem0.shape[1]
    seg = int(A_seg_len)
    HD = H * Dh
    T = S // CHUNKS
    assert T == SUB * SUBS and H == 4 * CHUNKS
    nt = D // LANES

    def rows(w):
        return jnp.transpose(w, (1, 2, 0)).reshape(HD, D)

    hbm = pl.BlockSpec(memory_space=pl.ANY)
    out = pl.pallas_call(
        functools.partial(_kernel, seg=seg, n_heads=H, dh=Dh),
        out_shape=jax.ShapeDtypeStruct((S, D), A_x.dtype),
        in_specs=[hbm] * 9,
        out_specs=hbm,
        scratch_shapes=[
            pltpu.VMEM((M, D), BF16),
            pltpu.VMEM((D,), BF16),
            pltpu.VMEM((S, D), BF16),
            pltpu.VMEM((4, HD, D), BF16),
            pltpu.VMEM((H // 2, D // 2, 6 * Dh), jnp.uint32),
            pltpu.VMEM((H // 2, Dh, D), jnp.uint32),
            pltpu.VMEM((3, D, D), BF16),
            pltpu.VMEM((D, D), BF16),
            pltpu.VMEM((nt, D, LANES), F32),
            pltpu.VMEM((3 * D // 2, D), jnp.uint32),
            pltpu.VMEM((D // 2, D), jnp.uint32),
            pltpu.VMEM((T, D), F32),
            pltpu.VMEM((nt, B_HIST + T, LANES), F32),
            pltpu.VMEM((nt, B_HIST + T, LANES), F32),
            pltpu.VMEM((T, D), BF16),
            pltpu.VMEM((S, D), F32),
            pltpu.VMEM((M + seg, D), F32),
            pltpu.VMEM((S, D), A_x.dtype),
            pltpu.SemaphoreType.DMA((7,)),
            pltpu.SemaphoreType.DMA((5 * CHUNKS,)),
            pltpu.SemaphoreType.DMA((1,)),
        ],
        compiler_params=pltpu.CompilerParams(vmem_limit_bytes=110 * 2**20),
    )(A_x.reshape(S, D), A_mem0.reshape(M, D), rows(A_Wq), rows(A_Wk), rows(A_Wv),
      A_Wo.reshape(HD, D), B_wqkv, B_wo, gate_w)
    return out.reshape(A_x.shape)
```

```python
import functools

import jax
import jax.numpy as jnp
from jax import lax
from jax.experimental import pallas as pl
from jax.experimental.pallas import tpu as pltpu

F32 = jnp.float32
BF16 = jnp.bfloat16
LANES = 128
NEG = -1000000000.0
LOG2E = 1.4426950408889634

B_HEADS = 32
B_WINDOW = 8
B_DIL = 2
B_HIST = 16
B_GROUP = 32

CHUNKS = 8
SUB = 128
SUBS = 2
LATE = 4
UNROLL = 3
LAG_SCORES, LAG_ATTEND, LAG_OUT = 1, 3, 5


def _dot(a, b):
    return lax.dot_general(a, b, (((1,), (0,)), ((), ())), preferred_element_type=F32)


def _dot_nt(a, b):
    return lax.dot_general(a, b, (((1,), (1,)), ((), ())), preferred_element_type=F32)


def _pack(a):
    return pltpu.bitcast(a, jnp.uint32)


def _unpack(a):
    return pltpu.bitcast(a, BF16)


def _kernel(x_hbm, mem0_hbm, wq_hbm, wk_hbm, wv_hbm, wo_hbm, bqkv_hbm, bwo_hbm, gw_hbm,
            out_hbm,
            mem0_ref, gw_ref, x_v, raw_v, w_v, wo_v, bqkv_v, bwo_v, perm_s, bqkv_p, bwo_p, q_s, k_s, v_s, ob_s,
            b_s, acc_s, out_v, sem_b, sem_w, sem_out, *, seg, n_heads, dh):
    S, D = x_v.shape
    M = mem0_ref.shape[0]
    L = M + seg
    n_seg = S // seg
    n_pairs = n_heads // 2
    pw = 2 * dh
    nt = D // LANES
    T = S // CHUNKS
    ppc = n_pairs // CHUNKS
    slab = ppc * pw
    w_hbm = (wq_hbm, wk_hbm, wv_hbm, wo_hbm)
    bdh = D // B_HEADS
    b_scale = bdh ** -0.5
    a_scale = dh ** -0.5

    def aligned(i, n):
        return i * n if isinstance(i, int) else pl.multiple_of(i * n, n)

    cp_bqkv = [pltpu.make_async_copy(bqkv_hbm.at[:, pl.ds(j * D, D)], bqkv_v.at[j],
                                     sem_b.at[4 + j]) for j in range(3)]
    cp_bwo = pltpu.make_async_copy(bwo_hbm, bwo_v, sem_b.at[1])

    cp_small = [pltpu.make_async_copy(mem0_hbm, mem0_ref, sem_b.at[2]),
                pltpu.make_async_copy(gw_hbm, gw_ref, sem_b.at[3])]

    def cp_x(c):
        rows = pl.ds(aligned(c, T), T)
        return pltpu.make_async_copy(x_hbm.at[rows], x_v.at[rows], sem_w.at[4 * CHUNKS + c])

    def cp_w(c):
        rows = pl.ds(aligned(c, slab), slab)
        return [pltpu.make_async_copy(w_hbm[j].at[rows], raw_v.at[j, rows],
                                      sem_w.at[j * CHUNKS + c]) for j in range(4)]

    def cp_out(s, n):
        rows = pl.ds(aligned(s, seg), n * seg)
        return pltpu.make_async_copy(out_v.at[rows], out_hbm.at[rows], sem_out.at[0])

    def start(copies):
        for cp in copies:
            cp.start()

    def wait(copies):
        for cp in copies:
            cp.wait()

    def reorder_rows(w, dst_ref, r0):
        wf = w.astype(F32)
        for t in range(nt):
            perm_s[t] = wf[:, t * LANES:(t + 1) * LANES]
        for d in range(bdh):
            blk = [perm_s[t, pl.ds(d, B_HEADS, stride=bdh), :] for t in range(nt)]
            o0 = (r0 + d * B_HEADS) // 2
            dst_ref[o0:o0 + B_HEADS // 2, :] = _pack(jnp.concatenate(blk, axis=1).astype(BF16))

    def b_project(c, u, j, is_first):
        xc = x_v[pl.ds(aligned(c * SUBS + u, SUB), SUB), :]
        z = _dot_nt(xc, _unpack(bqkv_p[j * D // 2:(j + 1) * D // 2, :]))
        if j == 0:
            q_s[u * SUB:(u + 1) * SUB, :] = z
            return
        ref = k_s if j == 1 else v_s
        o0 = B_HIST + u * SUB
        for t in range(nt):
            zt = z[:, t * LANES:(t + 1) * LANES]
            if u == 0 and is_first:
                ref[t, 0:B_HIST, :] = jnp.broadcast_to(zt[0:1, :], (B_HIST, LANES))
            elif u == 0:
                ref[t, 0:B_HIST, :] = ref[t, T:T + B_HIST, :]
            ref[t, o0:o0 + SUB, :] = zt

    def b_attend(g0, is_first):
        G = B_GROUP

        def windows(ref, t):
            views = {}
            for r in range(0, 8, B_DIL):
                shifts = range(r, B_WINDOW * B_DIL, 8)
                back = shifts[-1]
                o0 = B_HIST + g0 - back
                z = ref[t, o0:o0 + G + back - r, :]
                for sft in shifts:
                    views[sft // B_DIL] = z[back - sft:back - sft + G, :]
            return views

        logits = [None] * B_WINDOW
        for t in range(nt):
            qt = q_s[g0:g0 + G, t * LANES:(t + 1) * LANES]
            for w, kw in windows(k_s, t).items():
                logits[w] = qt * kw if t == 0 else logits[w] + qt * kw
        for w in range(B_WINDOW):
            acc = logits[w]
            sh = LANES // 2
            while sh >= B_HEADS:
                acc = acc + pltpu.roll(acc, sh, 1)
                sh //= 2
            if is_first and g0 < w * B_DIL:
                pos = g0 + lax.broadcasted_iota(jnp.int32, (G, LANES), 0)
                acc = jnp.where(pos >= w * B_DIL, acc, NEG / b_scale)
            logits[w] = acc
        mx = functools.reduce(jnp.maximum, logits)
        es = [jnp.exp2((l - mx) * (b_scale * LOG2E)) for l in logits]
        inv = 1.0 / functools.reduce(jnp.add, es)
        for t in range(nt):
            terms = [es[w] * vw for w, vw in windows(v_s, t).items()]
            acc = functools.reduce(jnp.add, terms) * inv
            ob_s[g0:g0 + G, t * LANES:(t + 1) * LANES] = acc.astype(BF16)

    def b_output(c, u):
        rows = pl.ds(aligned(c * SUBS + u, SUB), SUB)
        b_s[rows, :] = _dot(ob_s[u * SUB:(u + 1) * SUB, :], _unpack(bwo_p[...]))

    def relayout(c):
        for u in range(ppc):
            p = c * ppc + u
            rows = pl.ds(aligned(p, pw), pw)
            for j in range(3):
                w_v[p, :, j * pw:(j + 1) * pw] = _pack(raw_v[j, rows, :].T)
            wo_v[p] = _pack(raw_v[3, rows, :])

    def split_pair(z):
        col = lax.broadcasted_iota(jnp.int32, z.shape, 1)
        return jnp.concatenate([jnp.where(col < dh, z, 0.0), jnp.where(col >= dh, z, 0.0)],
                               axis=0).astype(BF16)

    def a_project(h, p):
        return _dot(h, _unpack(w_v[p]))

    def a_scores(qkv):
        return _dot_nt(qkv[:, 0:pw], split_pair(qkv[:, pw:2 * pw]))

    def a_attend(qkv, sc):
        row = lax.broadcasted_iota(jnp.int32, (L, 2 * L), 0)
        col = lax.broadcasted_iota(jnp.int32, (L, 2 * L), 1)
        in_a = col < L
        visible = (row < M) | (row >= jnp.where(in_a, col, col - L))
        sc = jnp.where(visible, sc * a_scale, NEG)
        ma = jnp.max(jnp.where(in_a, sc, -jnp.inf), axis=1, keepdims=True)
        mb = jnp.max(jnp.where(in_a, -jnp.inf, sc), axis=1, keepdims=True)
        e = jnp.exp(sc - jnp.where(in_a, ma, mb))
        la = jnp.sum(jnp.where(in_a, e, 0.0), axis=1, keepdims=True)
        lb = jnp.sum(jnp.where(in_a, 0.0, e), axis=1, keepdims=True)
        pr = e * (1.0 / jnp.where(in_a, la, lb))
        return _dot(pr, split_pair(qkv[:, 2 * pw:3 * pw]))

    def a_output(o, p, cols=slice(None)):
        return _dot(o, _unpack(wo_v[p, :, cols]))

    def a_tokens(s, mem):
        xs = x_v[pl.ds(aligned(s, seg), seg), :].astype(F32)
        return jnp.concatenate([mem, xs], axis=0)

    def finish(s, acc):
        rows = pl.ds(aligned(s, seg), seg)
        xs = x_v[rows, :].astype(F32)
        g = jax.nn.sigmoid(jnp.sum(xs * gw_ref[...].astype(F32).reshape(1, D), axis=1, keepdims=True))
        out_v[rows, :] = (g * acc[M:, :] + (1.0 - g) * b_s[rows, :]).astype(out_v.dtype)
        return acc[:M, :]

    def warmup(cb, ca):
        first = ca is None
        nb = 0 if cb is None else SUBS
        pairs = [] if ca is None else [ca * ppc + u for u in range(ppc)]
        if pairs:
            relayout(ca)
            h = a_tokens(0, mem0_ref[...].astype(F32))
        qkv, sc, o = {}, {}, {}
        pending = []

        def drain(n):
            for _ in range(min(n, len(pending))):
                b_attend(pending.pop(0), first)

        gps = SUB // B_GROUP
        for u in range(nb):
            for n, j in enumerate((1, 2, 0)):
                b_project(cb, u, j, first)
                drain(gps * (n + 1) // 3 - gps * n // 3)
            pending.extend(range(u * SUB, (u + 1) * SUB, B_GROUP))
        if pairs:
            qkv[0] = a_project(h, pairs[0])
            drain(gps // 2)
            qkv[1] = a_project(h, pairs[1])
            drain(gps)
            sc[0] = a_scores(qkv[0])
            sc[1] = a_scores(qkv[1])
        for u in range(nb // 2):
            b_output(cb, u)
            drain(-(-gps // (nb // 2)))
        if pairs:
            o[0] = a_attend(qkv[0], sc[0])
            o[1] = a_attend(qkv[1], sc[1])
        for u in range(nb // 2, nb):
            b_output(cb, u)
        if pairs:
            acc_s[...] += a_output(o[0], pairs[0]) + a_output(o[1], pairs[1])

    cp_bqkv[0].start()
    cp_bqkv[1].start()
    start(cp_small)
    acc_s[...] = jnp.zeros(acc_s.shape, F32)
    cp_bqkv[0].wait()
    cp_bqkv[2].start()
    cp_x(0).start()
    reorder_rows(bqkv_v[0].T, bqkv_p, 0)
    cp_bqkv[1].wait()
    cp_bwo.start()
    cp_x(1).start()
    reorder_rows(bqkv_v[1].T, bqkv_p, D)
    cp_bqkv[2].wait()
    start(cp_w(0))
    reorder_rows(bqkv_v[2].T, bqkv_p, 2 * D)
    cp_bwo.wait()
    cp_x(0).wait()
    wait(cp_small)
    cp_x(2).start()
    start(cp_w(1))
    reorder_rows(bwo_v[...], bwo_p, 0)
    warmup(0, None)

    def warmup_step(c, carry):
        cp_x(c).wait()
        wait(cp_w(c - 1))

        @pl.when(c + 2 < CHUNKS)
        def _():
            cp_x(c + 2).start()

        @pl.when(c + 1 < CHUNKS)
        def _():
            start(cp_w(c + 1))

        warmup(c, c - 1)
        return carry

    lax.fori_loop(1, CHUNKS, warmup_step, 0)
    wait(cp_w(CHUNKS - 1))
    warmup(None, CHUNKS - 1)
    mem1 = finish(0, acc_s[...])
    cp_out(0, 1).start()

    def accumulate(box, term):
        box[:] = [box[0] + term if box else term]

    def step(s, mem):
        h = a_tokens(s, mem)
        qkv, sc, o = {}, {}, {}
        head, last = [], []
        cut = D - LANES
        late = []
        for i in range(n_pairs + LAG_OUT):
            if i < n_pairs:
                qkv[i] = a_project(h, i)
            p = i - LAG_SCORES
            if 0 <= p < n_pairs:
                sc[p] = a_scores(qkv[p])
            p = i - LAG_OUT
            if 0 <= p < n_pairs:
                if p < n_pairs - LATE:
                    term = a_output(o.pop(p), p)
                    accumulate(head, term[:, :cut])
                    accumulate(last, term[:, cut:])
                else:
                    accumulate(head, a_output(o[p], p, slice(0, cut)))
                    late.append(p)
            p = i - LAG_ATTEND
            if 0 <= p < n_pairs:
                o[p] = a_attend(qkv.pop(p), sc.pop(p))
        for p in late:
            accumulate(last, a_output(o.pop(p), p, slice(cut, D)))
        return finish(s, jnp.concatenate([head[0], last[0]], axis=1))

    def steps(i, mem):
        s0 = 1 + i * UNROLL
        for u in range(UNROLL):
            mem = step(s0 + u, mem)
        cp_out(s0, UNROLL).start()
        return mem

    assert (n_seg - 1) % UNROLL == 0
    lax.fori_loop(0, (n_seg - 1) // UNROLL, steps, mem1)
    pltpu.make_async_copy(out_v, out_hbm, sem_out.at[0]).wait()


@functools.partial(jax.jit, static_argnames=("A_seg_len",))
def pallas_gated_mix__memory_aug_recurrent_mem_tr__sliding_local_dilated__prompt_kernel(
    A_x, A_mem0, A_Wq, A_Wk, A_Wv, A_Wo, A_seg_len, B_x, B_wqkv, B_wo, gate_w,
):
    del B_x
    _, S, D = A_x.shape
    _, H, Dh = A_Wq.shape
    M = A_mem0.shape[1]
    seg = int(A_seg_len)
    HD = H * Dh
    T = S // CHUNKS
    assert T == SUB * SUBS and H == 4 * CHUNKS
    nt = D // LANES

    def rows(w):
        return jnp.transpose(w, (1, 2, 0)).reshape(HD, D)

    hbm = pl.BlockSpec(memory_space=pl.ANY)
    out = pl.pallas_call(
        functools.partial(_kernel, seg=seg, n_heads=H, dh=Dh),
        out_shape=jax.ShapeDtypeStruct((S, D), A_x.dtype),
        in_specs=[hbm] * 9,
        out_specs=hbm,
        scratch_shapes=[
            pltpu.VMEM((M, D), BF16),
            pltpu.VMEM((D,), BF16),
            pltpu.VMEM((S, D), BF16),
            pltpu.VMEM((4, HD, D), BF16),
            pltpu.VMEM((H // 2, D // 2, 6 * Dh), jnp.uint32),
            pltpu.VMEM((H // 2, Dh, D), jnp.uint32),
            pltpu.VMEM((3, D, D), BF16),
            pltpu.VMEM((D, D), BF16),
            pltpu.VMEM((nt, D, LANES), F32),
            pltpu.VMEM((3 * D // 2, D), jnp.uint32),
            pltpu.VMEM((D // 2, D), jnp.uint32),
            pltpu.VMEM((T, D), F32),
            pltpu.VMEM((nt, B_HIST + T, LANES), F32),
            pltpu.VMEM((nt, B_HIST + T, LANES), F32),
            pltpu.VMEM((T, D), BF16),
            pltpu.VMEM((S, D), F32),
            pltpu.VMEM((M + seg, D), F32),
            pltpu.VMEM((S, D), A_x.dtype),
            pltpu.SemaphoreType.DMA((7,)),
            pltpu.SemaphoreType.DMA((5 * CHUNKS,)),
            pltpu.SemaphoreType.DMA((1,)),
        ],
        compiler_params=pltpu.CompilerParams(vmem_limit_bytes=110 * 2**20),
    )(A_x.reshape(S, D), A_mem0.reshape(M, D), rows(A_Wq), rows(A_Wk), rows(A_Wv),
      A_Wo.reshape(HD, D), B_wqkv, B_wo, gate_w)
    return out.reshape(A_x.shape)
```

```python
import functools

import jax
import jax.numpy as jnp
from jax import lax
from jax.experimental import pallas as pl
from jax.experimental.pallas import tpu as pltpu

F32 = jnp.float32
BF16 = jnp.bfloat16
LANES = 128
NEG = -1000000000.0
LOG2E = 1.4426950408889634

B_HEADS = 32
B_WINDOW = 8
B_DIL = 2
B_HIST = 16
B_GROUP = 32

CHUNKS = 8
SUB = 128
SUBS = 2
LATE = 4
UNROLL = 3
LAG_SCORES, LAG_ATTEND, LAG_OUT = 1, 3, 5


def _dot(a, b):
    return lax.dot_general(a, b, (((1,), (0,)), ((), ())), preferred_element_type=F32)


def _dot_nt(a, b):
    return lax.dot_general(a, b, (((1,), (1,)), ((), ())), preferred_element_type=F32)


def _pack(a):
    return pltpu.bitcast(a, jnp.uint32)


def _unpack(a):
    return pltpu.bitcast(a, BF16)


def _kernel(x_hbm, mem0_hbm, wq_hbm, wk_hbm, wv_hbm, wo_hbm, bqkv_hbm, bwo_hbm, gw_hbm,
            out_hbm,
            mem0_ref, gw_ref, x_v, raw_v, w_v, wo_v, bqkv_v, bwo_v, perm_s, bqkv_p, bwo_p,
            q_s, k_s, v_s, ob_s, b_s, acc_s, out_v, sem_b, sem_w, sem_out,
            *, seg, n_heads, dh):
    S, D = x_v.shape
    M = mem0_ref.shape[0]
    L = M + seg
    n_seg = S // seg
    n_pairs = n_heads // 2
    pw = 2 * dh
    nt = D // LANES
    T = S // CHUNKS
    ppc = n_pairs // CHUNKS
    slab = ppc * pw
    w_hbm = (wq_hbm, wk_hbm, wv_hbm, wo_hbm)
    bdh = D // B_HEADS
    b_scale = bdh ** -0.5
    a_scale = dh ** -0.5

    def aligned(i, n):
        return i * n if isinstance(i, int) else pl.multiple_of(i * n, n)

    cp_bqkv = [pltpu.make_async_copy(bqkv_hbm.at[:, pl.ds(j * D, D)], bqkv_v.at[j],
                                     sem_b.at[4 + j]) for j in range(3)]
    cp_bwo = pltpu.make_async_copy(bwo_hbm, bwo_v, sem_b.at[1])

    cp_small = [pltpu.make_async_copy(mem0_hbm, mem0_ref, sem_b.at[2]),
                pltpu.make_async_copy(gw_hbm, gw_ref, sem_b.at[3])]

    def cp_x(c):
        rows = pl.ds(aligned(c, T), T)
        return pltpu.make_async_copy(x_hbm.at[rows], x_v.at[rows], sem_w.at[4 * CHUNKS + c])

    def cp_w(c):
        rows = pl.ds(aligned(c, slab), slab)
        return [pltpu.make_async_copy(w_hbm[j].at[rows], raw_v.at[j, rows],
                                      sem_w.at[j * CHUNKS + c]) for j in range(4)]

    def cp_out(s, n):
        rows = pl.ds(aligned(s, seg), n * seg)
        return pltpu.make_async_copy(out_v.at[rows], out_hbm.at[rows], sem_out.at[0])

    def start(copies):
        for cp in copies:
            cp.start()

    def wait(copies):
        for cp in copies:
            cp.wait()

    def reorder_rows(w, dst_ref, r0):
        wf = w.astype(F32)
        for t in range(nt):
            perm_s[t, 0:D, :] = wf[:, t * LANES:(t + 1) * LANES]
        for d in range(bdh):
            blk = [perm_s[t, pl.ds(d, B_HEADS, stride=bdh), :] for t in range(nt)]
            o0 = (r0 + d * B_HEADS) // 2
            dst_ref[o0:o0 + B_HEADS // 2, :] = _pack(jnp.concatenate(blk, axis=1).astype(BF16))

    def b_project(c, u, j, is_first):
        xc = x_v[pl.ds(aligned(c * SUBS + u, SUB), SUB), :]
        z = _dot_nt(xc, _unpack(bqkv_p[j * D // 2:(j + 1) * D // 2, :]))
        if j == 0:
            q_s[u * SUB:(u + 1) * SUB, :] = z
            return
        ref = k_s if j == 1 else v_s
        o0 = B_HIST + u * SUB
        for t in range(nt):
            zt = z[:, t * LANES:(t + 1) * LANES]
            if u == 0 and is_first:
                ref[t, 0:B_HIST, :] = jnp.broadcast_to(zt[0:1, :], (B_HIST, LANES))
            elif u == 0:
                ref[t, 0:B_HIST, :] = ref[t, T:T + B_HIST, :]
            ref[t, o0:o0 + SUB, :] = zt

    def b_attend(g0, is_first):
        G = B_GROUP

        def windows(ref, t):
            views = {}
            for r in range(0, 8, B_DIL):
                shifts = range(r, B_WINDOW * B_DIL, 8)
                back = shifts[-1]
                o0 = B_HIST + g0 - back
                z = ref[t, o0:o0 + G + back - r, :]
                for sft in shifts:
                    views[sft // B_DIL] = z[back - sft:back - sft + G, :]
            return views

        logits = [None] * B_WINDOW
        for t in range(nt):
            qt = q_s[g0:g0 + G, t * LANES:(t + 1) * LANES]
            for w, kw in windows(k_s, t).items():
                logits[w] = qt * kw if t == 0 else logits[w] + qt * kw
        for w in range(B_WINDOW):
            acc = logits[w]
            sh = LANES // 2
            while sh >= B_HEADS:
                acc = acc + pltpu.roll(acc, sh, 1)
                sh //= 2
            if is_first and g0 < w * B_DIL:
                pos = g0 + lax.broadcasted_iota(jnp.int32, (G, LANES), 0)
                acc = jnp.where(pos >= w * B_DIL, acc, NEG / b_scale)
            logits[w] = acc
        mx = functools.reduce(jnp.maximum, logits)
        es = [jnp.exp2((l - mx) * (b_scale * LOG2E)) for l in logits]
        inv = 1.0 / functools.reduce(jnp.add, es)
        for t in range(nt):
            terms = [es[w] * vw for w, vw in windows(v_s, t).items()]
            acc = functools.reduce(jnp.add, terms) * inv
            ob_s[g0:g0 + G, t * LANES:(t + 1) * LANES] = acc.astype(BF16)

    def b_output(c, u):
        rows = pl.ds(aligned(c * SUBS + u, SUB), SUB)
        b_s[rows, :] = _dot(ob_s[u * SUB:(u + 1) * SUB, :], _unpack(bwo_p[...]))

    def relayout(c):
        for u in range(ppc):
            p = c * ppc + u
            rows = pl.ds(aligned(p, pw), pw)
            for j in range(3):
                w_v[p, :, j * pw:(j + 1) * pw] = _pack(raw_v[j, rows, :].T)
            wo_v[p] = _pack(raw_v[3, rows, :])

    def split_pair(z):
        col = lax.broadcasted_iota(jnp.int32, z.shape, 1)
        return jnp.concatenate([jnp.where(col < dh, z, 0.0), jnp.where(col >= dh, z, 0.0)],
                               axis=0).astype(BF16)

    def a_project(h, p):
        return _dot(h, _unpack(w_v[p]))

    def a_scores(qkv):
        return _dot_nt(qkv[:, 0:pw], split_pair(qkv[:, pw:2 * pw]))

    def a_attend(qkv, sc):
        row = lax.broadcasted_iota(jnp.int32, (L, 2 * L), 0)
        col = lax.broadcasted_iota(jnp.int32, (L, 2 * L), 1)
        in_a = col < L
        visible = (row < M) | (row >= jnp.where(in_a, col, col - L))
        sc = jnp.where(visible, sc * a_scale, NEG)
        ma = jnp.max(jnp.where(in_a, sc, -jnp.inf), axis=1, keepdims=True)
        mb = jnp.max(jnp.where(in_a, -jnp.inf, sc), axis=1, keepdims=True)
        e = jnp.exp(sc - jnp.where(in_a, ma, mb))
        la = jnp.sum(jnp.where(in_a, e, 0.0), axis=1, keepdims=True)
        lb = jnp.sum(jnp.where(in_a, 0.0, e), axis=1, keepdims=True)
        pr = e * (1.0 / jnp.where(in_a, la, lb))
        return _dot(pr, split_pair(qkv[:, 2 * pw:3 * pw]))

    def a_output(o, p, cols=slice(None)):
        return _dot(o, _unpack(wo_v[p, :, cols]))

    def a_tokens(s, mem):
        xs = x_v[pl.ds(aligned(s, seg), seg), :].astype(F32)
        return jnp.concatenate([mem, xs], axis=0)

    def finish(s, acc):
        rows = pl.ds(aligned(s, seg), seg)
        xs = x_v[rows, :].astype(F32)
        g = jax.nn.sigmoid(jnp.sum(xs * gw_ref[...].astype(F32).reshape(1, D), axis=1, keepdims=True))
        out_v[rows, :] = (g * acc[M:, :] + (1.0 - g) * b_s[rows, :]).astype(out_v.dtype)
        return acc[:M, :]

    def warmup(cb, ca):
        first = ca is None
        nb = 0 if cb is None else SUBS
        pairs = [] if ca is None else [ca * ppc + u for u in range(ppc)]
        if pairs:
            relayout(ca)
            h = a_tokens(0, mem0_ref[...].astype(F32))
        qkv, sc, o = {}, {}, {}
        pending = []

        def drain(n):
            for _ in range(min(n, len(pending))):
                b_attend(pending.pop(0), first)

        gps = SUB // B_GROUP
        for u in range(nb):
            for n, j in enumerate((1, 2, 0)):
                b_project(cb, u, j, first)
                drain(gps * (n + 1) // 3 - gps * n // 3)
            pending.extend(range(u * SUB, (u + 1) * SUB, B_GROUP))
        if pairs:
            qkv[0] = a_project(h, pairs[0])
            drain(gps // 2)
            qkv[1] = a_project(h, pairs[1])
            drain(gps)
            sc[0] = a_scores(qkv[0])
            sc[1] = a_scores(qkv[1])
        for u in range(nb // 2):
            b_output(cb, u)
            drain(-(-gps // (nb // 2)))
        if pairs:
            o[0] = a_attend(qkv[0], sc[0])
            o[1] = a_attend(qkv[1], sc[1])
        for u in range(nb // 2, nb):
            b_output(cb, u)
        if pairs:
            acc_s[...] += a_output(o[0], pairs[0]) + a_output(o[1], pairs[1])

    cp_bqkv[0].start()
    cp_bqkv[1].start()
    start(cp_small)
    acc_s[...] = jnp.zeros(acc_s.shape, F32)
    cp_bqkv[0].wait()
    cp_bqkv[2].start()
    cp_x(0).start()
    reorder_rows(bqkv_v[0].T, bqkv_p, 0)
    cp_bqkv[1].wait()
    cp_bwo.start()
    cp_x(1).start()
    reorder_rows(bqkv_v[1].T, bqkv_p, D)
    cp_bqkv[2].wait()
    start(cp_w(0))
    reorder_rows(bqkv_v[2].T, bqkv_p, 2 * D)
    cp_bwo.wait()
    cp_x(0).wait()
    wait(cp_small)
    cp_x(2).start()
    start(cp_w(1))
    reorder_rows(bwo_v[...], bwo_p, 0)
    warmup(0, None)

    def warmup_step(c, carry):
        cp_x(c).wait()
        wait(cp_w(c - 1))

        @pl.when(c + 2 < CHUNKS)
        def _():
            cp_x(c + 2).start()

        @pl.when(c + 1 < CHUNKS)
        def _():
            start(cp_w(c + 1))

        warmup(c, c - 1)
        return carry

    lax.fori_loop(1, CHUNKS, warmup_step, 0)
    wait(cp_w(CHUNKS - 1))
    warmup(None, CHUNKS - 1)
    mem1 = finish(0, acc_s[...])
    cp_out(0, 1).start()

    def accumulate(box, term):
        box[:] = [box[0] + term if box else term]

    def step(s, mem):
        h = a_tokens(s, mem)
        qkv, sc, o = {}, {}, {}
        head, last = [], []
        cut = D - LANES
        late = []
        for i in range(n_pairs + LAG_OUT):
            if i < n_pairs:
                qkv[i] = a_project(h, i)
            p = i - LAG_SCORES
            if 0 <= p < n_pairs:
                sc[p] = a_scores(qkv[p])
            p = i - LAG_OUT
            if 0 <= p < n_pairs:
                if p < n_pairs - LATE:
                    term = a_output(o.pop(p), p)
                    accumulate(head, term[:, :cut])
                    accumulate(last, term[:, cut:])
                else:
                    accumulate(head, a_output(o[p], p, slice(0, cut)))
                    late.append(p)
            p = i - LAG_ATTEND
            if 0 <= p < n_pairs:
                o[p] = a_attend(qkv.pop(p), sc.pop(p))
        for p in late:
            accumulate(last, a_output(o.pop(p), p, slice(cut, D)))
        return finish(s, jnp.concatenate([head[0], last[0]], axis=1))

    def steps(i, mem):
        s0 = 1 + i * UNROLL
        for u in range(UNROLL):
            mem = step(s0 + u, mem)
        cp_out(s0, UNROLL).start()
        return mem

    assert (n_seg - 1) % UNROLL == 0
    lax.fori_loop(0, (n_seg - 1) // UNROLL, steps, mem1)
    pltpu.make_async_copy(out_v, out_hbm, sem_out.at[0]).wait()


@functools.partial(jax.jit, static_argnames=("A_seg_len",))
def pallas_gated_mix__memory_aug_recurrent_mem_tr__sliding_local_dilated__prompt_kernel(
    A_x, A_mem0, A_Wq, A_Wk, A_Wv, A_Wo, A_seg_len, B_x, B_wqkv, B_wo, gate_w,
):
    del B_x
    _, S, D = A_x.shape
    _, H, Dh = A_Wq.shape
    M = A_mem0.shape[1]
    seg = int(A_seg_len)
    HD = H * Dh
    T = S // CHUNKS
    assert T == SUB * SUBS and H == 4 * CHUNKS
    nt = D // LANES

    def rows(w):
        return jnp.transpose(w, (1, 2, 0)).reshape(HD, D)

    hbm = pl.BlockSpec(memory_space=pl.ANY)
    out = pl.pallas_call(
        functools.partial(_kernel, seg=seg, n_heads=H, dh=Dh),
        out_shape=jax.ShapeDtypeStruct((S, D), A_x.dtype),
        in_specs=[hbm] * 9,
        out_specs=hbm,
        scratch_shapes=[
            pltpu.VMEM((M, D), BF16),
            pltpu.VMEM((D,), BF16),
            pltpu.VMEM((S, D), BF16),
            pltpu.VMEM((4, HD, D), BF16),
            pltpu.VMEM((H // 2, D // 2, 6 * Dh), jnp.uint32),
            pltpu.VMEM((H // 2, Dh, D), jnp.uint32),
            pltpu.VMEM((3, D, D), BF16),
            pltpu.VMEM((D, D), BF16),
            pltpu.VMEM((nt, D + 24, LANES), F32),
            pltpu.VMEM((3 * D // 2, D), jnp.uint32),
            pltpu.VMEM((D // 2, D), jnp.uint32),
            pltpu.VMEM((T, D), F32),
            pltpu.VMEM((nt, B_HIST + T, LANES), F32),
            pltpu.VMEM((nt, B_HIST + T, LANES), F32),
            pltpu.VMEM((T, D), BF16),
            pltpu.VMEM((S, D), F32),
            pltpu.VMEM((M + seg, D), F32),
            pltpu.VMEM((S, D), A_x.dtype),
            pltpu.SemaphoreType.DMA((7,)),
            pltpu.SemaphoreType.DMA((5 * CHUNKS,)),
            pltpu.SemaphoreType.DMA((1,)),
        ],
        compiler_params=pltpu.CompilerParams(vmem_limit_bytes=110 * 2**20),
    )(A_x.reshape(S, D), A_mem0.reshape(M, D), rows(A_Wq), rows(A_Wk), rows(A_Wv),
      A_Wo.reshape(HD, D), B_wqkv, B_wo, gate_w)
    return out.reshape(A_x.shape)
```
